```python
import os as _os
_os.environ.setdefault("JAX_PLATFORMS", "cpu")
import jax
import jax.numpy as jnp

def _softmax(x, axis=-1):
    return jax.nn.softmax(x, axis=axis)
def _gelu(x):
    return jax.nn.gelu(x, approximate=True)
def _silu(x):
    return jax.nn.silu(x)
def _sigmoid(x):
    return jax.nn.sigmoid(x)
def _layernorm(x, axis=-1, eps=1e-5):
    m = jnp.mean(x, axis=axis, keepdims=True)
    v = jnp.var(x, axis=axis, keepdims=True)
    return (x - m) / jnp.sqrt(v + eps)
def _scatter_add(tgt, idx, src, axis=0):
    return tgt.at[idx].add(src)
def _segment_sum(src, seg, n):
    return jax.ops.segment_sum(src, seg, n)
class _Rng:
    def __init__(self, key):
        self._k = key
    def _next(self):
        self._k, sub = jax.random.split(self._k)
        return sub
    def normal(self, shape):
        return jax.random.normal(self._next(), shape, dtype=jnp.bfloat16)
    def randint(self, lo, hi, shape):
        return jax.random.randint(self._next(), shape, lo, hi, dtype=jnp.int32)
    def uniform(self, shape, lo=0.0, hi=1.0):
        return jax.random.uniform(self._next(), shape, jnp.bfloat16, lo, hi)
    def permutation(self, n):
        return jax.random.permutation(self._next(), n)


kernel_name = 'standalone__dense_activation_silu__prompt'

def setup_inputs():
    _rng = _Rng(jax.random.key(int.from_bytes(__import__("os").urandom(4), "little")))
    _w = (lambda a: (lambda t: t.astype(jnp.bfloat16) if jnp.issubdtype(t.dtype, jnp.floating) else t)(jnp.asarray(a)))
    B, S, D, F = 1, 2048, 448, 1792
    return {
        "x": _w((lambda *s: _rng.normal(s) * 0.05)(B, S, D)),
        "w1": _w((lambda *s: _rng.normal(s) * 0.05)(D, F) * (D ** -0.5)),
        "w2": _w((lambda *s: _rng.normal(s) * 0.05)(F, D) * (F ** -0.5)),
    }

def reference(x, w1, w2):
    h = jnp.einsum("bsd,df->bsf", x, w1)
    h = _silu(h)
    out = jnp.einsum("bsf,fd->bsd", h, w2)
    return out
```

```python
import jax
import jax.numpy as jnp
import jax.experimental.pallas as pl
import jax.experimental.pallas.tpu as pltpu

_STAGES = ((256, 384), (512, 640), (1024, 1152))
_TILE = 256
_LAST_SPLIT = 4


def _silu(h):
    hh = 0.5 * h
    return hh + hh * jnp.tanh(hh)


@jax.jit
def pallas_standalone__dense_activation_silu__prompt_kernel(
    x: jax.Array,
    w1: jax.Array,
    w2: jax.Array,
):
    B, S0, D = x.shape
    F = w1.shape[1]
    S = B * S0
    dt = x.dtype
    f32 = jnp.float32
    ng = len(_STAGES) + 1

    def kernel(x_hbm, w1_hbm, w2_hbm, o_hbm, xs, w1s, w2s, w1t, os_, hs, sem):
        def col_copy(src, dst, c0, c1, g):
            return pltpu.make_async_copy(
                src.at[:, pl.ds(c0, c1 - c0)], dst.at[:, pl.ds(c0, c1 - c0)], sem.at[g])

        groups = []
        pa = pb = 0
        for g, (a, b) in enumerate(_STAGES):
            groups.append([col_copy(w1_hbm, w1s, pb, b, g), col_copy(x_hbm, xs, pa, a, g)])
            pa, pb = a, b
        groups.append([col_copy(w1_hbm, w1s, pb, F, ng - 1), col_copy(w2_hbm, w2s, 0, F, ng - 1),
                       col_copy(x_hbm, xs, pa, S, ng - 1)])
        for grp in groups:
            for c in grp:
                c.start()

        stores = []

        def transpose_w1(f0, f1):
            v = w1s[:, f0:f1].T
            w1t[f0:f1, :] = v
            return v

        def up(lhs, f0, f1, s0, s1):
            h = jnp.dot(lhs, xs[:, s0:s1], preferred_element_type=f32)
            hs[f0:f1, s0:s1] = _silu(h).astype(dt)

        def down(h, s0, s1):
            acc = jnp.dot(w2s[...], h, preferred_element_type=f32)
            n = _LAST_SPLIT if s1 == S else 1
            r = D // n
            for j in range(n):
                os_[j * r:(j + 1) * r, s0:s1] = acc[j * r:(j + 1) * r].astype(dt)
                c = pltpu.make_async_copy(
                    os_.at[pl.ds(j * r, r), pl.ds(s0, s1 - s0)],
                    o_hbm.at[pl.ds(j * r, r), pl.ds(s0, s1 - s0)], sem.at[ng])
                c.start()
                stores.append(c)

        pa = pb = 0
        for g, (a, b) in enumerate(_STAGES):
            for c in groups[g]:
                c.wait()
            if pb:
                up(w1t[0:pb, :], 0, pb, pa, a)
            up(transpose_w1(pb, b), pb, b, 0, a)
            pa, pb = a, b
        for c in groups[ng - 1]:
            c.wait()
        up(w1t[0:pb, :], 0, pb, pa, pa + _TILE)
        v = transpose_w1(pb, F)
        for s0 in range(0, pa + _TILE, _TILE):
            up(v if s0 == 0 else w1t[pb:F, :], pb, F, s0, s0 + _TILE)
            down(hs[:, s0:s0 + _TILE], s0, s0 + _TILE)
        for s0 in range(pa + _TILE, S, _TILE):
            h = jnp.dot(w1t[...], xs[:, s0:s0 + _TILE], preferred_element_type=f32)
            down(_silu(h).astype(dt), s0, s0 + _TILE)
        for c in stores:
            c.wait()

    xt = x.reshape(S, D).T
    ot = pl.pallas_call(
        kernel,
        in_specs=[pl.BlockSpec(memory_space=pl.ANY)] * 3,
        out_specs=pl.BlockSpec(memory_space=pl.ANY),
        out_shape=jax.ShapeDtypeStruct((D, S), dt),
        scratch_shapes=[
            pltpu.VMEM((D, S), dt), pltpu.VMEM((D, F), dt), pltpu.VMEM((D, F), dt),
            pltpu.VMEM((F, D), dt), pltpu.VMEM((D, S), dt), pltpu.VMEM((F, S), dt),
            pltpu.SemaphoreType.DMA((ng + 1,)),
        ],
        compiler_params=pltpu.CompilerParams(vmem_limit_bytes=64 * 1024 * 1024),
    )(xt, w1, w2.T)
    return ot.T.reshape(B, S0, D)
```

```python
import jax
import jax.numpy as jnp
import jax.experimental.pallas as pl
import jax.experimental.pallas.tpu as pltpu
from jax import lax

_LANES = 128
_NUM_PARTS = 2
_PIECES = (
    ("w", 2), ("x", 1), ("x", 1), ("x", 1), ("w", 1), ("x", 1),
    ("w", 2), ("x", 2), ("w", 2), ("w", 3), ("x", 2), ("w", 4),
)
_OUT_TILES = (4, 2, 2)
_LAST_TILE_SLABS = 4


def _silu(h):
    d = 1.0 + jnp.exp(-h)
    r = pl.reciprocal(d, approx=True)
    r = r * (2.0 - d * r)
    return h * jnp.where(d < jnp.inf, r, 0.0)


@jax.jit
def pallas_standalone__dense_activation_silu__prompt_kernel(
    x: jax.Array,
    w1: jax.Array,
    w2: jax.Array,
):
    batch, seq, d_model = x.shape
    d_ff = w1.shape[1]
    rows = batch * seq
    part = rows // _NUM_PARTS
    dtype = x.dtype

    pieces = []
    done = {"w": 0, "x": 0}
    for kind, n in _PIECES:
        pieces.append((kind, done[kind], done[kind] + n * _LANES))
        done[kind] += n * _LANES
    assert done == {"w": d_ff, "x": part} and pieces[0][0] == "w"

    slabs = []
    c0 = 0
    for n in _OUT_TILES:
        c1 = c0 + n * _LANES
        k = _LAST_TILE_SLABS if c1 == part else 1
        r = d_model // k
        slabs.append([(q * r, (q + 1) * r, c0, c1) for q in range(k)])
        c0 = c1
    assert c0 == part and d_model % (16 * _LAST_TILE_SLABS) == 0

    sem_w2, sem_x, sem_out = len(pieces), len(pieces) + 1, len(pieces) + 2

    def kernel(x_hbm, w1_hbm, w2_hbm, y_hbm, x_v, w1_v, w2_v, w1t_v, h_v, y_v, sems):
        loads = []
        for g, (kind, a, b) in enumerate(pieces):
            cols = pl.ds(a, b - a)
            src, dst = (w1_hbm, w1_v) if kind == "w" else (x_hbm, x_v.at[0])
            loads.append(
                pltpu.make_async_copy(src.at[:, cols], dst.at[:, cols], sems.at[g]))
        late_loads = [pltpu.make_async_copy(w2_hbm, w2_v, sems.at[sem_w2])]
        for p in range(1, _NUM_PARTS):
            late_loads.append(
                pltpu.make_async_copy(
                    x_hbm.at[:, pl.ds(p * part, part)], x_v.at[p], sems.at[sem_x]))
        for copy in loads + late_loads:
            copy.start()

        def store(p, slab):
            r0, r1, s0, s1 = slab
            col = p * part + s0
            if not isinstance(col, int):
                col = pl.multiple_of(col, _LANES)
            return pltpu.make_async_copy(
                y_v.at[pl.ds(r0, r1 - r0), pl.ds(s0, s1 - s0)],
                y_hbm.at[pl.ds(r0, r1 - r0), pl.ds(col, s1 - s0)],
                sems.at[sem_out])

        def wait_stores(p):
            for tile in slabs:
                for slab in tile:
                    store(p, slab).wait()

        def transpose_w1(f0, f1):
            w1t_v[f0:f1, :] = w1_v[:, f0:f1].T

        loads[0].wait()
        transpose_w1(pieces[0][1], pieces[0][2])

        def do_part(p, carry):
            def up(f0, f1, s0, s1):
                h = jnp.dot(w1t_v[f0:f1, :], x_v[p, :, s0:s1],
                            preferred_element_type=jnp.float32)
                h_v[f0:f1, s0:s1] = _silu(h).astype(dtype)

            num_x, num_w = 0, pieces[0][2]
            for copy, (kind, a, b) in zip(loads[1:], pieces[1:]):
                pl.when(p == 0)(copy.wait)
                if kind == "w":
                    transpose_w1(a, b)
                    up(a, b, 0, num_x)
                    num_w = b
                else:
                    up(0, num_w, a, b)
                    num_x = b
            for copy in late_loads:
                pl.when(p == 0)(copy.wait)

            for t, tile in enumerate(slabs):
                s0, s1 = tile[0][2], tile[0][3]
                acc = None
                for k0 in range(0, d_ff, _LANES):
                    term = jnp.dot(w2_v[:, k0:k0 + _LANES], h_v[k0:k0 + _LANES, s0:s1],
                                   preferred_element_type=jnp.float32)
                    acc = term if acc is None else acc + term
                if t == 0:
                    pl.when(p > 0)(lambda: wait_stores(p - 1))
                for slab in tile:
                    r0, r1 = slab[0], slab[1]
                    y_v[r0:r1, s0:s1] = acc[r0:r1].astype(dtype)
                    store(p, slab).start()
            return carry

        lax.fori_loop(0, _NUM_PARTS, do_part, None)
        wait_stores(_NUM_PARTS - 1)

    y_t = pl.pallas_call(
        kernel,
        in_specs=[pl.BlockSpec(memory_space=pl.ANY)] * 3,
        out_specs=pl.BlockSpec(memory_space=pl.ANY),
        out_shape=jax.ShapeDtypeStruct((d_model, rows), dtype),
        scratch_shapes=[
            pltpu.VMEM((_NUM_PARTS, d_model, part), dtype),
            pltpu.VMEM((d_model, d_ff), dtype),
            pltpu.VMEM((d_model, d_ff), dtype),
            pltpu.VMEM((d_ff, d_model), dtype),
            pltpu.VMEM((d_ff, part), dtype),
            pltpu.VMEM((d_model, part), dtype),
            pltpu.SemaphoreType.DMA((sem_out + 1,)),
        ],
        compiler_params=pltpu.CompilerParams(
            vmem_limit_bytes=64 * 1024 * 1024,
            disable_semaphore_checks=True,
            flags={"XLA_TPU_RESCHEDULE_DMA_DONES": True},
        ),
    )(x.reshape(rows, d_model).T, w1, w2.T)
    return y_t.T.reshape(batch, seq, d_model)
```

```python
import jax
import jax.numpy as jnp
import jax.experimental.pallas as pl
import jax.experimental.pallas.tpu as pltpu
from jax import lax

_LANES = 128
_LOG2_E = 1.4426950408889634
_NUM_PARTS = 2
_PIECES = (
    ("w", 2), ("x", 2), ("x", 1), ("x", 1), ("x", 1),
    ("w", 1), ("x", 3), ("w", 3), ("w", 3), ("w", 5),
)
_OUT_TILES = (6, 2)
_LAST_TILE_SLABS = 14


def _silu(h):
    d = 1.0 + jnp.exp2(h * -_LOG2_E)
    r = pl.reciprocal(d, approx=True)
    t = h * r
    return jnp.where(d < jnp.inf, t * (2.0 - d * r), t)


@jax.jit
def pallas_standalone__dense_activation_silu__prompt_kernel(
    x: jax.Array,
    w1: jax.Array,
    w2: jax.Array,
):
    batch, seq, d_model = x.shape
    d_ff = w1.shape[1]
    rows = batch * seq
    part = rows // _NUM_PARTS
    dtype = x.dtype

    pieces = []
    done = {"w": 0, "x": 0}
    for kind, n in _PIECES:
        pieces.append((kind, done[kind], done[kind] + n * _LANES))
        done[kind] += n * _LANES
    assert done == {"w": d_ff, "x": part} and pieces[0][0] == "w"

    slabs = []
    c0 = 0
    for n in _OUT_TILES:
        c1 = c0 + n * _LANES
        k = _LAST_TILE_SLABS if c1 == part else 1
        r = d_model // k
        slabs.append([(q * r, (q + 1) * r, c0, c1) for q in range(k)])
        c0 = c1
    assert c0 == part and d_model % (16 * _LAST_TILE_SLABS) == 0

    sem_w2, sem_x, sem_out = len(pieces), len(pieces) + 1, len(pieces) + 2

    def kernel(x_hbm, w1_hbm, w2_hbm, y_hbm, x_v, w1_v, w2_v, w1t_v, h_v, y_v, sems):
        loads = []
        for g, (kind, a, b) in enumerate(pieces):
            cols = pl.ds(a, b - a)
            src, dst = (w1_hbm, w1_v) if kind == "w" else (x_hbm, x_v.at[0])
            loads.append(
                pltpu.make_async_copy(src.at[:, cols], dst.at[:, cols], sems.at[g]))
        late_loads = [pltpu.make_async_copy(w2_hbm, w2_v, sems.at[sem_w2])]
        for p in range(1, _NUM_PARTS):
            late_loads.append(
                pltpu.make_async_copy(
                    x_hbm.at[:, pl.ds(p * part, part)], x_v.at[p], sems.at[sem_x]))
        for copy in loads + late_loads:
            copy.start()

        def store(p, slab):
            r0, r1, s0, s1 = slab
            col = p * part + s0
            if not isinstance(col, int):
                col = pl.multiple_of(col, _LANES)
            return pltpu.make_async_copy(
                y_v.at[pl.ds(r0, r1 - r0), pl.ds(s0, s1 - s0)],
                y_hbm.at[pl.ds(r0, r1 - r0), pl.ds(col, s1 - s0)],
                sems.at[sem_out])

        def wait_stores(p):
            for tile in slabs:
                for slab in tile:
                    store(p, slab).wait()

        def transpose_w1(f0, f1):
            w1t_v[f0:f1, :] = w1_v[:, f0:f1].T

        loads[0].wait()
        transpose_w1(pieces[0][1], pieces[0][2])

        def do_part(p, carry):
            def up(f0, f1, s0, s1):
                h = jnp.dot(w1t_v[f0:f1, :], x_v[p, :, s0:s1],
                            preferred_element_type=jnp.float32)
                h_v[f0:f1, s0:s1] = _silu(h).astype(dtype)

            num_x, num_w = 0, pieces[0][2]
            for copy, (kind, a, b) in zip(loads[1:], pieces[1:]):
                pl.when(p == 0)(copy.wait)
                if kind == "w":
                    transpose_w1(a, b)
                    up(a, b, 0, num_x)
                    num_w = b
                else:
                    up(0, num_w, a, b)
                    num_x = b
            for copy in late_loads:
                pl.when(p == 0)(copy.wait)

            for t, tile in enumerate(slabs):
                s0, s1 = tile[0][2], tile[0][3]
                acc = None
                for k0 in range(0, d_ff, _LANES):
                    term = jnp.dot(w2_v[:, k0:k0 + _LANES], h_v[k0:k0 + _LANES, s0:s1],
                                   preferred_element_type=jnp.float32)
                    acc = term if acc is None else acc + term
                if t == 0:
                    pl.when(p > 0)(lambda: wait_stores(p - 1))
                for slab in tile:
                    r0, r1 = slab[0], slab[1]
                    y_v[r0:r1, s0:s1] = acc[r0:r1].astype(dtype)
                    store(p, slab).start()
            return carry

        lax.fori_loop(0, _NUM_PARTS, do_part, None)
        wait_stores(_NUM_PARTS - 1)

    y_t = pl.pallas_call(
        kernel,
        in_specs=[pl.BlockSpec(memory_space=pl.ANY)] * 3,
        out_specs=pl.BlockSpec(memory_space=pl.ANY),
        out_shape=jax.ShapeDtypeStruct((d_model, rows), dtype),
        scratch_shapes=[
            pltpu.VMEM((_NUM_PARTS, d_model, part), dtype),
            pltpu.VMEM((d_model, d_ff), dtype),
            pltpu.VMEM((d_model, d_ff), dtype),
            pltpu.VMEM((d_ff, d_model), dtype),
            pltpu.VMEM((d_ff, part), dtype),
            pltpu.VMEM((d_model, part), dtype),
            pltpu.SemaphoreType.DMA((sem_out + 1,)),
        ],
        compiler_params=pltpu.CompilerParams(
            vmem_limit_bytes=64 * 1024 * 1024,
            disable_semaphore_checks=True,
            flags={"XLA_TPU_RESCHEDULE_DMA_DONES": True},
        ),
    )(x.reshape(rows, d_model).T, w1, w2.T)
    return y_t.T.reshape(batch, seq, d_model)
```
